```python
import os as _os
_os.environ.setdefault("JAX_PLATFORMS", "cpu")
import jax
import jax.numpy as jnp

def _softmax(x, axis=-1):
    return jax.nn.softmax(x, axis=axis)
def _gelu(x):
    return jax.nn.gelu(x, approximate=True)
def _silu(x):
    return jax.nn.silu(x)
def _sigmoid(x):
    return jax.nn.sigmoid(x)
def _layernorm(x, axis=-1, eps=1e-5):
    m = jnp.mean(x, axis=axis, keepdims=True)
    v = jnp.var(x, axis=axis, keepdims=True)
    return (x - m) / jnp.sqrt(v + eps)
def _scatter_add(tgt, idx, src, axis=0):
    return tgt.at[idx].add(src)
def _segment_sum(src, seg, n):
    return jax.ops.segment_sum(src, seg, n)
class _Rng:
    def __init__(self, key):
        self._k = key
    def _next(self):
        self._k, sub = jax.random.split(self._k)
        return sub
    def normal(self, shape):
        return jax.random.normal(self._next(), shape, dtype=jnp.bfloat16)
    def randint(self, lo, hi, shape):
        return jax.random.randint(self._next(), shape, lo, hi, dtype=jnp.int32)
    def uniform(self, shape, lo=0.0, hi=1.0):
        return jax.random.uniform(self._next(), shape, jnp.bfloat16, lo, hi)
    def permutation(self, n):
        return jax.random.permutation(self._next(), n)


kernel_name = 'standalone__mha_softmax__near_ridge'

def setup_inputs():
    _rng = _Rng(jax.random.key(int.from_bytes(__import__("os").urandom(4), "little")))
    _w = (lambda a: (lambda t: t.astype(jnp.bfloat16) if jnp.issubdtype(t.dtype, jnp.floating) else t)(jnp.asarray(a)))
    B, H, Sq, Sk, D = 8, 16, 192, 1024, 256
    return {
        "q": _w((lambda *s: _rng.normal(s) * 0.4)(B, H, Sq, D)),
        "k": _w((lambda *s: _rng.normal(s) * 0.4)(B, H, Sk, D)),
        "v": _w((lambda *s: _rng.normal(s) * 0.05)(B, H, Sk, D)),
    }

def reference(q, k, v):
    scale = q.shape[-1] ** -0.5
    scores = jnp.einsum("bhqd,bhkd->bhqk", q, k) * scale
    p = _softmax(scores, axis=-1)
    return jnp.einsum("bhqk,bhkd->bhqd", p, v)
```

```python
import math

import jax
import jax.numpy as jnp
from jax import lax
import jax.experimental.pallas as pl
import jax.experimental.pallas.tpu as pltpu

GROUP = 4
RING = 3
LOOKAHEAD = GROUP + 2
READ_ROWS = 64
WRITE_ROWS = 128
LOG2E = math.log2(math.e)


def _attention_head(q, k, v, scale):
    s = lax.dot_general(
        q, k, (((1,), (1,)), ((), ())), preferred_element_type=jnp.float32
    )
    m = jnp.max(s, axis=-1, keepdims=True)
    p = jnp.exp2((s - m) * (scale * LOG2E))
    l = jnp.sum(p, axis=-1, keepdims=True)
    o = jnp.dot(p.astype(v.dtype), v, preferred_element_type=jnp.float32)
    return o * (1.0 / l)


@jax.jit
def pallas_standalone__mha_softmax__near_ridge_kernel(
    q: jax.Array,
    k: jax.Array,
    v: jax.Array,
):
    B, H, SQ, D = q.shape
    SK = k.shape[2]
    scale = D**-0.5
    n = B * H
    n_groups = n // GROUP
    chunks = SK // (READ_ROWS * GROUP)
    q_rows = SQ // 2
    writes_per_step = (n - LOOKAHEAD) // LOOKAHEAD
    assert n % GROUP == 0 and chunks * READ_ROWS * GROUP == SK
    assert LOOKAHEAD <= (RING - 1) * GROUP and LOOKAHEAD < n
    assert SQ % 32 == 0 and SQ > WRITE_ROWS

    def kernel(q_hbm, k_hbm, v_hbm, o_hbm, q_buf, k_buf, v_buf, o_buf, in_sems, o_sem):
        def head_of(group, member):
            return member * n_groups + group

        def fetch_part(part):
            group, sub = part // GROUP, part % GROUP
            slot = group % RING
            for c in range(chunks):
                rows = pl.ds(
                    pl.multiple_of((sub * chunks + c) * READ_ROWS, READ_ROWS),
                    READ_ROWS,
                )
                for member in range(GROUP):
                    head = head_of(group, member)
                    pltpu.make_async_copy(
                        k_hbm.at[head, rows],
                        k_buf.at[slot, member, rows],
                        in_sems.at[1, slot],
                    ).start(priority=0)
                    pltpu.make_async_copy(
                        v_hbm.at[head, rows],
                        v_buf.at[slot, member, rows],
                        in_sems.at[2, slot],
                    ).start(priority=1)
            for c in range(2):
                rows = pl.ds(c * q_rows, q_rows)
                pltpu.make_async_copy(
                    q_hbm.at[head_of(group, sub), rows],
                    q_buf.at[slot, sub, rows],
                    in_sems.at[0, slot],
                ).start(priority=c)

        def wait_group(slot):
            for a, buf in enumerate((q_buf, k_buf, v_buf)):
                pltpu.make_async_copy(
                    buf.at[slot], buf.at[slot], in_sems.at[a, slot]
                ).wait()

        def write_back(step, _):
            head = head_of(step // GROUP, step % GROUP)
            for c, rows in enumerate(
                (pl.ds(0, WRITE_ROWS), pl.ds(WRITE_ROWS, SQ - WRITE_ROWS))
            ):
                pltpu.make_async_copy(
                    o_buf.at[step, rows], o_hbm.at[head, rows], o_sem.at[0]
                ).start(priority=c)

        def compute_step(i, _):
            group, member = i // GROUP, i % GROUP
            slot = group % RING

            @pl.when(i + LOOKAHEAD < n)
            def _():
                fetch_part(i + LOOKAHEAD)

            @pl.when(i + LOOKAHEAD >= n)
            def _():
                first = (i + LOOKAHEAD - n) * writes_per_step
                lax.fori_loop(first, first + writes_per_step, write_back, None)

            @pl.when(member == 0)
            def _():
                wait_group(slot)

            o_buf[i] = _attention_head(
                q_buf[slot, member], k_buf[slot, member], v_buf[slot, member], scale
            ).astype(o_buf.dtype)

        lax.fori_loop(0, LOOKAHEAD, lambda part, _: fetch_part(part), None)
        lax.fori_loop(0, n, compute_step, None)
        lax.fori_loop(LOOKAHEAD * writes_per_step, n, write_back, None)
        pltpu.make_async_copy(o_buf, o_buf, o_sem.at[0]).wait()

    out = pl.pallas_call(
        kernel,
        in_specs=[pl.BlockSpec(memory_space=pl.ANY)] * 3,
        out_specs=pl.BlockSpec(memory_space=pl.ANY),
        out_shape=jax.ShapeDtypeStruct((n, SQ, D), q.dtype),
        scratch_shapes=[
            pltpu.VMEM((RING, GROUP, SQ, D), q.dtype),
            pltpu.VMEM((RING, GROUP, SK, D), k.dtype),
            pltpu.VMEM((RING, GROUP, SK, D), v.dtype),
            pltpu.VMEM((n, SQ, D), q.dtype),
            pltpu.SemaphoreType.DMA((3, RING)),
            pltpu.SemaphoreType.DMA((1,)),
        ],
        compiler_params=pltpu.CompilerParams(
            vmem_limit_bytes=64 << 20,
            disable_bounds_checks=True,
        ),
    )(q.reshape(n, SQ, D), k.reshape(n, SK, D), v.reshape(n, SK, D))
    return out.reshape(B, H, SQ, D)
```

```python
import math

import jax
import jax.numpy as jnp
from jax import lax
import jax.experimental.pallas as pl
import jax.experimental.pallas.tpu as pltpu

GROUP = 4
RING = 3
LOOKAHEAD = GROUP + 2
COPY_ROWS = 64
WRITE_STREAMS = 8
LOG2E = math.log2(math.e)


def _attention_head(q, k, v, scale):
    s = lax.dot_general(
        q, k, (((1,), (1,)), ((), ())), preferred_element_type=jnp.float32
    )
    m = jnp.max(s, axis=-1, keepdims=True)
    p = jnp.exp2((s - m) * (scale * LOG2E))
    l = jnp.sum(p, axis=-1, keepdims=True)
    o = jnp.dot(p.astype(v.dtype), v, preferred_element_type=jnp.float32)
    return o * (1.0 / l)


def _copy_rows(start):
    if not isinstance(start, int):
        start = pl.multiple_of(start, COPY_ROWS)
    return pl.ds(start, COPY_ROWS)


@jax.jit
def pallas_standalone__mha_softmax__near_ridge_kernel(
    q: jax.Array,
    k: jax.Array,
    v: jax.Array,
):
    B, H, SQ, D = q.shape
    SK = k.shape[2]
    scale = D**-0.5
    n = B * H
    n_groups = n // GROUP
    kv_copies = SK // (COPY_ROWS * GROUP)
    q_copies = SQ // COPY_ROWS
    units = n // WRITE_STREAMS
    units_per_step = units // (LOOKAHEAD + 2)

    assert q.dtype == k.dtype == v.dtype
    assert n % GROUP == 0 and n % WRITE_STREAMS == 0 and n > LOOKAHEAD
    assert kv_copies * COPY_ROWS * GROUP == SK
    assert q_copies * COPY_ROWS == SQ and q_copies <= GROUP
    assert GROUP - 1 <= LOOKAHEAD <= (RING - 1) * GROUP
    for t in range(LOOKAHEAD):
        for unit in range(t * units_per_step, (t + 1) * units_per_step):
            for stream in range(WRITE_STREAMS):
                group = (stream * units + unit) % n_groups
                assert (group + 1) * GROUP <= n - LOOKAHEAD + t

    def kernel(q_hbm, k_hbm, v_hbm, o_hbm, in_buf, o_buf, sems):

        def head_of(group, member):
            return member * n_groups + group

        def fetch_part(part):
            if isinstance(part, int):
                group, sub = divmod(part, GROUP)
                slot = group % RING
            else:
                group, sub = lax.div(part, GROUP), lax.rem(part, GROUP)
                slot = lax.rem(group, RING)

            def fetch(src, member, row, dst_offset, priority):
                pltpu.make_async_copy(
                    src.at[head_of(group, member), _copy_rows(row)],
                    in_buf.at[slot, member, _copy_rows(dst_offset + row)],
                    sems.at[slot],
                ).start(priority=priority)

            for c in range(kv_copies):
                row = (sub * kv_copies + c) * COPY_ROWS
                for member in range(GROUP):
                    fetch(k_hbm, member, row, 0, priority=0)
                    fetch(v_hbm, member, row, SK, priority=1)

            @pl.when(sub < q_copies)
            def _():
                for member in range(GROUP):
                    fetch(q_hbm, member, sub * COPY_ROWS, 2 * SK, member % 2)

        def write_unit(unit, _):
            for c in range(q_copies):
                rows = _copy_rows(c * COPY_ROWS)
                for stream in range(WRITE_STREAMS):
                    head = stream * units + unit
                    pltpu.make_async_copy(
                        o_buf.at[head, rows], o_hbm.at[head, rows], sems.at[RING]
                    ).start(priority=stream % 2)

        def step(i, _):
            group, member = lax.div(i, GROUP), lax.rem(i, GROUP)
            slot = lax.rem(group, RING)

            @pl.when(i + LOOKAHEAD < n)
            def _():
                fetch_part(i + LOOKAHEAD)

            @pl.when(i + LOOKAHEAD >= n)
            def _():
                first = (i + LOOKAHEAD - n) * units_per_step
                lax.fori_loop(first, first + units_per_step, write_unit, None)

            @pl.when(member == 0)
            def _():
                pltpu.make_async_copy(
                    in_buf.at[slot], in_buf.at[slot], sems.at[slot]
                ).wait()

            out = _attention_head(
                in_buf[slot, member, pl.ds(2 * SK, SQ)],
                in_buf[slot, member, pl.ds(0, SK)],
                in_buf[slot, member, pl.ds(SK, SK)],
                scale,
            )
            o_buf[head_of(group, member)] = out.astype(o_buf.dtype)

        fetch_part(0)
        lax.fori_loop(1, LOOKAHEAD, lambda part, _: fetch_part(part), None)
        lax.fori_loop(0, n, step, None)
        lax.fori_loop(LOOKAHEAD * units_per_step, units, write_unit, None)
        pltpu.make_async_copy(o_buf, o_hbm, sems.at[RING]).wait()

    out = pl.pallas_call(
        kernel,
        in_specs=[pl.BlockSpec(memory_space=pl.ANY)] * 3,
        out_specs=pl.BlockSpec(memory_space=pl.ANY),
        out_shape=jax.ShapeDtypeStruct((n, SQ, D), q.dtype),
        scratch_shapes=[
            pltpu.VMEM((RING, GROUP, 2 * SK + SQ, D), q.dtype),
            pltpu.VMEM((n, SQ, D), q.dtype),
            pltpu.SemaphoreType.DMA((RING + 1,)),
        ],
        compiler_params=pltpu.CompilerParams(
            vmem_limit_bytes=64 << 20,
            disable_bounds_checks=True,
        ),
    )(q.reshape(n, SQ, D), k.reshape(n, SK, D), v.reshape(n, SK, D))
    return out.reshape(B, H, SQ, D)
```
